```python
import os as _os
_os.environ.setdefault("JAX_PLATFORMS", "cpu")
import jax
import jax.numpy as jnp

def _softmax(x, axis=-1):
    return jax.nn.softmax(x, axis=axis)
def _gelu(x):
    return jax.nn.gelu(x, approximate=True)
def _silu(x):
    return jax.nn.silu(x)
def _sigmoid(x):
    return jax.nn.sigmoid(x)
def _layernorm(x, axis=-1, eps=1e-5):
    m = jnp.mean(x, axis=axis, keepdims=True)
    v = jnp.var(x, axis=axis, keepdims=True)
    return (x - m) / jnp.sqrt(v + eps)
def _scatter_add(tgt, idx, src, axis=0):
    return tgt.at[idx].add(src)
def _segment_sum(src, seg, n):
    return jax.ops.segment_sum(src, seg, n)
class _Rng:
    def __init__(self, key):
        self._k = key
    def _next(self):
        self._k, sub = jax.random.split(self._k)
        return sub
    def normal(self, shape):
        return jax.random.normal(self._next(), shape, dtype=jnp.bfloat16)
    def randint(self, lo, hi, shape):
        return jax.random.randint(self._next(), shape, lo, hi, dtype=jnp.int32)
    def uniform(self, shape, lo=0.0, hi=1.0):
        return jax.random.uniform(self._next(), shape, jnp.bfloat16, lo, hi)
    def permutation(self, n):
        return jax.random.permutation(self._next(), n)


kernel_name = 'standalone__gqa_block_cached__near_ridge'

def setup_inputs():
    _rng = _Rng(jax.random.key(int.from_bytes(__import__("os").urandom(4), "little")))
    _w = (lambda a: (lambda t: t.astype(jnp.bfloat16) if jnp.issubdtype(t.dtype, jnp.floating) else t)(jnp.asarray(a)))
    B, Sq, D = 16, 128, 576
    Hq, Hkv, Sk, Dh = 32, 16, 1024, 128
    assert Hq % Hkv == 0, (Hq, Hkv)
    return {
        "x": _w((lambda *s: _rng.normal(s) * 0.8)(B, Sq, D)),
        "k_cache": _w((lambda *s: _rng.normal(s) * 0.8)(B, Hkv, Sk, Dh)),
        "v_cache": _w((lambda *s: _rng.normal(s) * 0.05)(B, Hkv, Sk, Dh)),
        "wq": _w((lambda *s: _rng.normal(s) * 0.8)(D, Hq * Dh) * (D ** -0.5)),
        "wo": _w((lambda *s: _rng.normal(s) * 0.05)(Hq * Dh, D) * ((Hq * Dh) ** -0.5)),
    }

def reference(x, k_cache, v_cache, wq, wo):
    B, Sq, D = x.shape
    Hq, Dh = 32, 128
    Hkv = k_cache.shape[1]
    rep = Hq // Hkv
    q = (lambda x, *d: x.transpose(*d))((x @ wq).reshape(B, Sq, Hq, Dh), 0, 2, 1, 3)
    k = jnp.repeat(k_cache, rep, axis=1)
    v = jnp.repeat(v_cache, rep, axis=1)
    scores = jnp.einsum("bhqd,bhkd->bhqk", q, k) * (Dh ** -0.5)
    p = _softmax(scores, axis=-1)
    o = jnp.einsum("bhqk,bhkd->bhqd", p, v)
    return (lambda x, *d: x.transpose(*d))(o, 0, 2, 1, 3).reshape(B, Sq, Hq * Dh) @ wo
```

```python
import functools, math
import numpy as np
import jax
import jax.numpy as jnp
from jax import lax
from jax.experimental import pallas as pl
from jax.experimental.pallas import tpu as pltpu

NT = (((1,), (1,)), ((), ()))
f32 = jnp.float32
bf16 = jnp.bfloat16

def ld16(ref):
    return pltpu.bitcast(ref.bitcast(jnp.int32)[...], bf16)

def make(G=4, vmem=100, order='BBCBCBCCAE', flags=None, AM=4, RC=16, KS=2, U=1, nodma=False, interpret=False, pld=True, HH=16, abl='', mode='online', GS=4, NBUF=4, PD=2, N1=4, dorder='x0 q k0 v0 x1 x2 k1 v1 o w x3'):
    ldp = ld16 if pld else (lambda r: r[...])
    B, Sq, D, H, Sk, Dh = 16, 128, 576, 16, 1024, 128
    NG = B // G
    NI = HH * NG
    WD = NG + 1 + U
    HW = 2 * H + 4
    NS = max(NG - 1, 2)
    RP = D // (NG // 2)
    W = Sk // KS
    c = float(Dh ** -0.5 * math.log2(math.e))
    NK = -(-D // 128)

    def kernel(xT_hbm, k_hbm, v_hbm, wq_hbm, woT_hbm, out_hbm,
               xtbuf, xbuf, kbuf, vbuf, wqbuf, wobuf, qs, os_, acc, ostage, pbuf, rbuf, sbuf, mbuf,
               xsem, ksem, vsem, wqsem, wosem, osem):
        def mo(v, n):
            return v if isinstance(v, int) else pl.multiple_of(v, n)
        def kv_copies(i, which='kv', part=None):
            slot = i % NBUF
            ic = min(i, NI - 1) if isinstance(i, int) else jnp.minimum(i, NI - 1)
            h = ic // NG
            r = []
            for c_ in (range(G // GS) if part is None else [part]):
                b0 = (ic % NG) * G + c_ * GS
                if 'k' in which:
                    r.append(pltpu.make_async_copy(k_hbm.at[pl.ds(b0, GS), h], kbuf.at[slot, pl.ds(c_ * GS, GS)], ksem.at[slot, c_]))
                if 'v' in which:
                    r.append(pltpu.make_async_copy(v_hbm.at[pl.ds(b0, GS), h], vbuf.at[slot, pl.ds(c_ * GS, GS)], vsem.at[slot, c_]))
            return r
        def w_copies(n):
            hh = n // NG
            pc = n % NG
            j = pc % 2
            r0 = mo((pc // 2) * RP, RP)
            hs = min(hh, H - 1) if isinstance(hh, int) else jnp.minimum(hh, H - 1)
            col = mo((2 * hs + j) * Dh, Dh)
            par = n % 8
            return (pltpu.make_async_copy(wq_hbm.at[pl.ds(r0, RP), pl.ds(col, Dh)], wqbuf.at[2 * hh + j, pl.ds(r0, RP)], wqsem.at[par]),
                    pltpu.make_async_copy(woT_hbm.at[pl.ds(r0, RP), pl.ds(col, Dh)], wobuf.at[2 * hh + j, pl.ds(r0, RP)], wosem.at[par]))
        def w0_copies(src, dst, sem):
            return [pltpu.make_async_copy(src.at[:, pl.ds(j * Dh, Dh)], dst.at[j, pl.ds(0, D)], sem.at[8 + j]) for j in range(2)]
        def x_copy(g):
            return pltpu.make_async_copy(xT_hbm.at[pl.ds(g * G, G)], xtbuf.at[pl.ds(g * G, G)], xsem.at[g])
        def o_copy(b):
            return pltpu.make_async_copy(ostage.at[b], out_hbm.at[b], osem.at[b])

        def xpose_group(g):
            for p in range(G):
                b = g * G + p
                for k in range(NK):
                    rows = min(128, D - k * 128)
                    xt = ld16(xtbuf.at[b, pl.ds(k * 128, rows)])
                    if rows < 128:
                        xt = jnp.concatenate([xt, jnp.zeros((128 - rows, Sq), bf16)], axis=0)
                    xbuf[k, pl.ds(mo(b * Sq, Sq), Sq), :] = xt.T

        def stage_A(i, qslot):
            h = i // NG
            b0 = (i % NG) * G
            for a in range(G // AM):
                r0 = mo((b0 + a * AM) * Sq, AM * Sq)
                x = jnp.concatenate([ld16(xbuf.at[k, pl.ds(r0, AM * Sq)]) for k in range(NK)], axis=1)
                for j in range(2):
                    q = jnp.dot(x, ld16(wqbuf.at[2 * h + j]), preferred_element_type=f32)
                    q = (q * c).astype(bf16)
                    for p in range(AM):
                        qs[qslot, a * AM + p, pl.ds(j * Sq, Sq), :] = q[p * Sq:(p + 1) * Sq]

        NT_ = W // 128
        def lanefold(op, v):
            return functools.reduce(op, [v[:, t * 128:(t + 1) * 128] for t in range(v.shape[1] // 128)])

        def stage_B(p, slot, qslot):
            q = ld16(qs.at[qslot, p])
            if mode == 'twopassx':
                sl = (slot + p) % 2
                s = lax.dot_general(q, ld16(kbuf.at[slot, p]), NT, preferred_element_type=f32)
                for t in range(Sk // 128):
                    sbuf[sl, t] = s[:, t * 128:(t + 1) * 128]
                mbuf[sl] = lanefold(jnp.maximum, s)
                return sl
            return [lax.dot_general(q, ld16(kbuf.at[slot, p, pl.ds(u * W, W)]), NT, preferred_element_type=f32) for u in range(KS)]

        def stage_X(p, ss):
            if mode == 'twopassx':
                sl = ss
                for rc in range(2 * Sq // RC):
                    rows = pl.ds(rc * RC, RC)
                    m = jnp.max(mbuf[sl, rows, :], axis=1, keepdims=True)
                    l = None
                    for t in range(Sk // 128):
                        pr = jnp.exp2(sbuf[sl, t, rows, :] - m)
                        l = pr if l is None else l + pr
                        pbuf[p % 2, t, rows, :] = pr.astype(bf16)
                    l = jnp.sum(l, axis=1, keepdims=True)
                    r = pl.reciprocal(l, approx=True)
                    r = r * (2.0 - l * r)
                    rbuf[p % 2, 0, rows, :] = jnp.broadcast_to(r, (RC, Dh))
                return
            for rc in range(2 * Sq // RC):
                rows = slice(rc * RC, (rc + 1) * RC)
                if mode == 'twopass':
                    m = jnp.max(functools.reduce(jnp.maximum, [lanefold(jnp.maximum, t[rows]) for t in ss]), axis=1, keepdims=True)
                ms = []; ls = []
                for u in range(KS):
                    s = ss[u][rows]
                    if mode != 'twopass':
                        mu = jnp.max(s, axis=1, keepdims=True)
                        m = mu if u == 0 else jnp.maximum(m, mu)
                    pr = jnp.exp2(s - m)
                    ms.append(m)
                    ls.append(lanefold(jnp.add, pr))
                    pb = pr.astype(bf16)
                    for t in range(NT_):
                        pbuf[p % 2, u * NT_ + t, pl.ds(rc * RC, RC), :] = pb[:, t * 128:(t + 1) * 128]
                if mode == 'twopass':
                    l = jnp.sum(functools.reduce(jnp.add, ls), axis=1, keepdims=True)
                else:
                    al = [jnp.exp2(ms[u] - m) for u in range(KS - 1)]
                    l = ls[-1]
                    for u in range(KS - 1):
                        l = l + al[u] * ls[u]
                    l = jnp.sum(l, axis=1, keepdims=True)
                r = pl.reciprocal(l, approx=True)
                r = r * (2.0 - l * r)
                if mode == 'twopass':
                    rbuf[p % 2, 0, pl.ds(rc * RC, RC), :] = jnp.broadcast_to(r, (RC, Dh))
                else:
                    for u in range(KS):
                        ru = r if u == KS - 1 else r * al[u]
                        rbuf[p % 2, u, pl.ds(rc * RC, RC), :] = jnp.broadcast_to(ru, (RC, Dh))

        def stage_C(p, slot, oslot):
            if mode in ('twopass', 'twopassx'):
                pu = jnp.concatenate([ldp(pbuf.at[p % 2, t]) for t in range(Sk // 128)], axis=1)
                o = jnp.dot(pu, ld16(vbuf.at[slot, p]), preferred_element_type=f32) * rbuf[p % 2, 0]
            else:
                o = None
                for u in range(KS):
                    pu = jnp.concatenate([ldp(pbuf.at[p % 2, u * NT_ + t]) for t in range(NT_)], axis=1)
                    ou = jnp.dot(pu, ld16(vbuf.at[slot, p, pl.ds(u * W, W)]), preferred_element_type=f32) * rbuf[p % 2, u]
                    o = ou if o is None else o + ou
            os_[oslot, p] = o.astype(bf16)

        def stage_E(i, oslot, first=False):
            h = i // NG
            b0 = (i % NG) * G
            for p in range(G):
                y = lax.dot_general(ld16(wobuf.at[2 * h]), ld16(os_.at[oslot, p, pl.ds(0, Sq)]), NT, preferred_element_type=f32)
                y = y + lax.dot_general(ld16(wobuf.at[2 * h + 1]), ld16(os_.at[oslot, p, pl.ds(Sq, Sq)]), NT, preferred_element_type=f32)
                if isinstance(h, int):
                    acc[b0 + p] = y if h == 0 else acc[b0 + p] + y
                else:
                    acc[b0 + p] = jnp.where(h > 0, acc[b0 + p], 0.0) + y

        def emit_out(g):
            for p in range(G):
                b = g * G + p
                ostage[b] = acc[b].astype(bf16)
                o_copy(b).start()

        def step(i, kvw=(1,)):
            static = isinstance(i, int)
            first = static and i == 0
            early = static and i < NS
            last = static and i == NI - 1
            slot = i % NBUF
            qslot = i % 2
            cnt = dict(B=0, X=0, C=0, A=0, E=0, W=0, S=0)
            ss = {}; done = set()
            def do_starts():
                if first:
                    issue(3)
                if not last and not nodma:
                    for cp in kv_copies(i + PD):
                        cp.start()
                    for cp in w_copies(i + WD):
                        cp.start()
            def do_waits():
                if last or nodma or not kvw or (early and i < NS - 1):
                    return
                pieces = range(NG, i + WD) if early else [i + WD - 1 - d_ for d_ in range(len(kvw))]
                for n_ in pieces:
                    for cp in w_copies(n_):
                        cp.wait()
                for t_ in kvw:
                    for cp in kv_copies(i + t_):
                        cp.wait()
            if last:
                for g in range(NG - 2):
                    emit_out(g)
            for ch in order:
                n = cnt[ch]; cnt[ch] += 1
                if ch == 'B':
                    if early and n % GS == 0:
                        for cp in kv_copies(i, 'k', n // GS):
                            cp.wait()
                    ss[n] = stage_B(n, slot, qslot)
                    if n == 0 and 'S' not in order:
                        do_starts()
                elif ch == 'S':
                    do_starts()
                elif ch == 'W':
                    do_waits()
                elif ch == 'X':
                    stage_X(n, ss.pop(n)); done.add(n)
                elif ch == 'C':
                    if early and n % GS == 0:
                        for cp in kv_copies(i, 'v', n // GS):
                            cp.wait()
                    if n not in done:
                        stage_X(n, ss.pop(n))
                    stage_C(n, slot, qslot)
                elif ch == 'A':
                    if early and i + 1 < NG:
                        x_copy(i + 1).wait()
                        xpose_group(i + 1)
                    if not last and 'A' not in abl:
                        stage_A(i + 1, 1 - qslot)
                elif ch == 'E':
                    if static and i == 1:
                        for cp in w0_copies(woT_hbm, wobuf, wosem):
                            cp.wait()
                    if not first and 'E' not in abl:
                        stage_E(i - 1, 1 - qslot)
                    if last and NG > 1:
                        emit_out(NG - 2)
            if 'W' not in order:
                do_waits()

        items = dict(x0=[x_copy(0)], q=w0_copies(wq_hbm, wqbuf, wqsem), o=w0_copies(woT_hbm, wobuf, wosem),
                     k0=kv_copies(0, 'k'), v0=kv_copies(0, 'v'), **{'k%d' % t: kv_copies(t, 'k') for t in range(1, PD)}, **{'v%d' % t: kv_copies(t, 'v') for t in range(1, PD)}, w=[cp for n_ in range(NG, WD) for cp in w_copies(n_)],
                     **{'x%d' % g: [x_copy(g)] for g in range(1, NG)})
        parts = [p_.split() for p_ in dorder.split('|')]
        parts += [[]] * (4 - len(parts))
        assert sorted(sum(parts, [])) == sorted(items)
        def issue(k_):
            for nm in parts[k_]:
                for cp in items[nm]:
                    cp.start()
        issue(0)
        wqbuf[:, pl.ds(D, NK * 128 - D), :] = jnp.zeros((HW, NK * 128 - D, Dh), bf16)
        x_copy(0).wait()
        issue(1)
        xpose_group(0)
        for cp in w0_copies(wq_hbm, wqbuf, wqsem):
            cp.wait()
        stage_A(0, 0)
        issue(2)
        if nodma:
            for t in range(1, PD):
                for cp in kv_copies(t):
                    cp.wait()
            for cp in w_copies(NG):
                cp.wait()
        for i_ in range(NS):
            step(i_)
        n1 = N1 if U == 2 else NI - 2
        if 1 + n1 > NS:
            lax.fori_loop(NS, 1 + n1, lambda t, c_: (step(t), c_)[1], 0)
        if U == 2:
            assert (NI - 2 - n1) % 2 == 0
            for cp in kv_copies(n1 + 2):
                cp.wait()
            def body(t, carry):
                i = n1 + 1 + 2 * t
                step(i, ())
                step(i + 1, (1, 2))
                return carry
            lax.fori_loop(0, (NI - 2 - n1) // 2, body, 0)
        step(NI - 1)
        nwaited = NI if U == 1 else NI + 1
        for t in range(nwaited, NI - 1 + PD):
            for cp in kv_copies(t):
                cp.wait()
        for cp in w_copies(NI - 2 + WD):
            cp.wait()
        stage_E(NI - 1, (NI - 1) % 2)
        emit_out(NG - 1)
        for b in range(B):
            o_copy(b).wait()

    @jax.jit
    def pallas_standalone__gqa_block_cached__near_ridge_kernel(x, k_cache, v_cache, wq, wo):
        xT = x.transpose(0, 2, 1)
        woT = wo.T
        anyspec = pl.BlockSpec(memory_space=pl.ANY)
        outT = pl.pallas_call(
            kernel,
            in_specs=[anyspec] * 5,
            out_specs=anyspec,
            out_shape=jax.ShapeDtypeStruct((B, D, Sq), x.dtype),
            scratch_shapes=[
                pltpu.VMEM((B, D, Sq), bf16),
                pltpu.VMEM((NK, B * Sq, 128), bf16),
                pltpu.VMEM((NBUF, G, Sk, Dh), bf16),
                pltpu.VMEM((NBUF, G, Sk, Dh), bf16),
                pltpu.VMEM((HW, NK * 128, Dh), bf16),
                pltpu.VMEM((HW, D, Dh), bf16),
                pltpu.VMEM((2, G, 2 * Sq, Dh), bf16),
                pltpu.VMEM((2, G, 2 * Sq, Dh), bf16),
                pltpu.VMEM((B, D, Sq), f32),
                pltpu.VMEM((B, D, Sq), bf16),
                pltpu.VMEM((2, Sk // 128, 2 * Sq, 128), bf16),
                pltpu.VMEM((2, KS, 2 * Sq, Dh), f32),
                pltpu.VMEM((2, Sk // 128 if mode == 'twopassx' else 1, 2 * Sq, 128), f32),
                pltpu.VMEM((2, 2 * Sq, 128), f32),
                pltpu.SemaphoreType.DMA((NG,)),
                pltpu.SemaphoreType.DMA((NBUF, G // GS)),
                pltpu.SemaphoreType.DMA((NBUF, G // GS)),
                pltpu.SemaphoreType.DMA((10,)),
                pltpu.SemaphoreType.DMA((10,)),
                pltpu.SemaphoreType.DMA((B,)),
            ],
            compiler_params=pltpu.CompilerParams(vmem_limit_bytes=vmem * 1024 * 1024, **({'flags': flags} if flags else {})),
            interpret=interpret,
        )(xT, k_cache, v_cache, wq, woT)
        return outT.transpose(0, 2, 1)
    return pallas_standalone__gqa_block_cached__near_ridge_kernel


pallas_standalone__gqa_block_cached__near_ridge_kernel = make(AM=2,order='BESXBCXBCXBCXCA',U=2,PD=3,N1=2,dorder='x0 q k0 v0 x1 k1 v1 o x2 k2 v2 x3 w')
```

```python
import functools
import math
import numpy as np
import jax
import jax.numpy as jnp
from jax import lax
from jax.experimental import pallas as pl
from jax.experimental.pallas import tpu as pltpu

NT = (((1,), (1,)), ((), ()))
f32 = jnp.float32
bf16 = jnp.bfloat16

def ld16(ref):
    return pltpu.bitcast(ref.bitcast(jnp.int32)[...], bf16)

def _build():
    G, AM, RC, KS = 4, 2, 32, 2
    NBUF, PD, U, N1 = 4, 3, 2, 2
    order = 'BESXBCXBCXBCXCA'
    dorder = 'x0 q k0a v0a x1 o k1 v1 x2 k2 v2 x3 w'
    GS = G0 = G
    HH = 16
    vmem = 100
    ldp = ld16
    B, Sq, D, H, Sk, Dh = 16, 128, 576, 16, 1024, 128
    NG = B // G
    NI = HH * NG
    WD = NG + 1 + U
    HW = 2 * H + 4
    NS = max(NG - 1, 2)
    RP = D // (NG // 2)
    W = Sk // KS
    c = float(Dh ** -0.5 * math.log2(math.e))
    NK = -(-D // 128)

    def kernel(xT_hbm, k_hbm, v_hbm, wq_hbm, woT_hbm, out_hbm,
               xtbuf, xbuf, kbuf, vbuf, wqbuf, wobuf, qs, os_, acc, ostage, pbuf, rbuf,
               k0sem, xsem, ksem, vsem, wqsem, wosem, osem):
        def mo(v, n):
            return v if isinstance(v, int) else pl.multiple_of(v, n)
        def kv_copies(i, which='kv', part=None):
            slot = i % NBUF
            ic = min(i, NI - 1) if isinstance(i, int) else jnp.minimum(i, NI - 1)
            h = ic // NG
            r = []
            if isinstance(i, int) and i == 0:
                for c_ in (range(G // G0) if part is None else [part]):
                    if 'k' in which:
                        r.append(pltpu.make_async_copy(k_hbm.at[pl.ds(c_ * G0, G0), 0], kbuf.at[0, pl.ds(c_ * G0, G0)], k0sem.at[0, c_]))
                    if 'v' in which:
                        r.append(pltpu.make_async_copy(v_hbm.at[pl.ds(c_ * G0, G0), 0], vbuf.at[0, pl.ds(c_ * G0, G0)], k0sem.at[1, c_]))
                return r
            for c_ in (range(G // GS) if part is None else [part]):
                b0 = (ic % NG) * G + c_ * GS
                if 'k' in which:
                    r.append(pltpu.make_async_copy(k_hbm.at[pl.ds(b0, GS), h], kbuf.at[slot, pl.ds(c_ * GS, GS)], ksem.at[slot, c_]))
                if 'v' in which:
                    r.append(pltpu.make_async_copy(v_hbm.at[pl.ds(b0, GS), h], vbuf.at[slot, pl.ds(c_ * GS, GS)], vsem.at[slot, c_]))
            return r
        def w_copies(n):
            hh = n // NG
            pc = n % NG
            j = pc % 2
            r0 = mo((pc // 2) * RP, RP)
            hs = min(hh, H - 1) if isinstance(hh, int) else jnp.minimum(hh, H - 1)
            col = mo((2 * hs + j) * Dh, Dh)
            par = n % 8
            return (pltpu.make_async_copy(wq_hbm.at[pl.ds(r0, RP), pl.ds(col, Dh)], wqbuf.at[2 * hh + j, pl.ds(r0, RP)], wqsem.at[par]),
                    pltpu.make_async_copy(woT_hbm.at[pl.ds(r0, RP), pl.ds(col, Dh)], wobuf.at[2 * hh + j, pl.ds(r0, RP)], wosem.at[par]))
        def w0_copies(src, dst, sem):
            return [pltpu.make_async_copy(src.at[:, pl.ds(j * Dh, Dh)], dst.at[j, pl.ds(0, D)], sem.at[8 + j]) for j in range(2)]
        def x_copy(g):
            return pltpu.make_async_copy(xT_hbm.at[pl.ds(g * G, G)], xtbuf.at[pl.ds(g * G, G)], xsem.at[g])
        def o_copy(b):
            return pltpu.make_async_copy(ostage.at[b], out_hbm.at[b], osem.at[b])

        def xpose_group(g, ps=None):
            for p in (range(G) if ps is None else ps):
                b = g * G + p
                for k in range(NK):
                    rows = min(128, D - k * 128)
                    xt = ld16(xtbuf.at[b, pl.ds(k * 128, rows)])
                    if rows < 128:
                        xt = jnp.concatenate([xt, jnp.zeros((128 - rows, Sq), bf16)], axis=0)
                    xbuf[k, pl.ds(mo(b * Sq, Sq), Sq), :] = xt.T

        def stage_A(i, qslot):
            h = i // NG
            b0 = (i % NG) * G
            for a in range(G // AM):
                r0 = mo((b0 + a * AM) * Sq, AM * Sq)
                x = jnp.concatenate([ld16(xbuf.at[k, pl.ds(r0, AM * Sq)]) for k in range(NK)], axis=1)
                for j in range(2):
                    q = jnp.dot(x, ld16(wqbuf.at[2 * h + j]), preferred_element_type=f32)
                    q = (q * c).astype(bf16)
                    for p in range(AM):
                        qs[qslot, a * AM + p, pl.ds(j * Sq, Sq), :] = q[p * Sq:(p + 1) * Sq]

        NT_ = W // 128
        def lanefold(op, v):
            return functools.reduce(op, [v[:, t * 128:(t + 1) * 128] for t in range(v.shape[1] // 128)])

        def stage_B(p, slot, qslot):
            q = ld16(qs.at[qslot, p])
            return [lax.dot_general(q, ld16(kbuf.at[slot, p, pl.ds(u * W, W)]), NT, preferred_element_type=f32) for u in range(KS)]

        def stage_X(p, ss):
            for rc in range(2 * Sq // RC):
                rows = slice(rc * RC, (rc + 1) * RC)
                ms = []; ls = []
                for u in range(KS):
                    s = ss[u][rows]
                    mu = jnp.max(s, axis=1, keepdims=True)
                    m = mu if u == 0 else jnp.maximum(m, mu)
                    pr = jnp.exp2(s - m)
                    ms.append(m)
                    ls.append(lanefold(jnp.add, pr))
                    pb = pr.astype(bf16)
                    for t in range(NT_):
                        pbuf[p % 2, u * NT_ + t, pl.ds(rc * RC, RC), :] = pb[:, t * 128:(t + 1) * 128]
                al = [jnp.exp2(ms[u] - m) for u in range(KS - 1)]
                l = ls[-1]
                for u in range(KS - 1):
                    l = l + al[u] * ls[u]
                l = jnp.sum(l, axis=1, keepdims=True)
                r = pl.reciprocal(l, approx=True)
                r = r * (2.0 - l * r)
                for u in range(KS):
                    ru = r if u == KS - 1 else r * al[u]
                    rbuf[p % 2, u, pl.ds(rc * RC, RC), :] = jnp.broadcast_to(ru, (RC, Dh))

        def stage_C(p, slot, oslot):
            o = None
            for u in range(KS):
                pu = jnp.concatenate([ldp(pbuf.at[p % 2, u * NT_ + t]) for t in range(NT_)], axis=1)
                ou = jnp.dot(pu, ld16(vbuf.at[slot, p, pl.ds(u * W, W)]), preferred_element_type=f32) * rbuf[p % 2, u]
                o = ou if o is None else o + ou
            os_[oslot, p] = o.astype(bf16)

        def stage_E(i, oslot, final=False):
            h = i // NG
            b0 = (i % NG) * G
            for p in range(G):
                y = lax.dot_general(ld16(wobuf.at[2 * h]), ld16(os_.at[oslot, p, pl.ds(0, Sq)]), NT, preferred_element_type=f32)
                y = y + lax.dot_general(ld16(wobuf.at[2 * h + 1]), ld16(os_.at[oslot, p, pl.ds(Sq, Sq)]), NT, preferred_element_type=f32)
                if final:
                    ostage[b0 + p] = (acc[b0 + p] + y).astype(bf16)
                    o_copy(b0 + p).start()
                elif isinstance(h, int):
                    acc[b0 + p] = y if h == 0 else acc[b0 + p] + y
                else:
                    acc[b0 + p] = jnp.where(h > 0, acc[b0 + p], 0.0) + y

        def emit_out(g):
            for p in range(G):
                b = g * G + p
                ostage[b] = acc[b].astype(bf16)
                o_copy(b).start()

        def step(i, kvw=(1,)):
            static = isinstance(i, int)
            first = static and i == 0
            early = static and i < NS
            last = static and i == NI - 1
            slot = i % NBUF
            qslot = i % 2
            cnt = dict(B=0, X=0, C=0, A=0, E=0, W=0, S=0)
            ss = {}; done = set()
            def do_starts():
                if not last:
                    for cp in kv_copies(i + PD):
                        cp.start()
                    for cp in w_copies(i + WD):
                        cp.start()
            def do_waits():
                if last or not kvw:
                    return
                if early and i + 2 < NG:
                    x_copy(i + 2).wait()
                if first:
                    for cp in w0_copies(woT_hbm, wobuf, wosem):
                        cp.wait()
                if early and i < NS - 1:
                    for cp in kv_copies(i + 1):
                        cp.wait()
                    return
                pieces = range(NG, i + WD) if early else [i + WD - 1 - d_ for d_ in range(len(kvw))]
                for n_ in pieces:
                    for cp in w_copies(n_):
                        cp.wait()
                for t_ in kvw:
                    for cp in kv_copies(i + t_):
                        cp.wait()
            if last:
                for g in range(NG - 2):
                    emit_out(g)
            for ch in order:
                n = cnt[ch]; cnt[ch] += 1
                if ch == 'B':
                    gs_ = G0 if first else GS
                    if first and n % gs_ == 0:
                        for cp in kv_copies(i, 'k', n // gs_):
                            cp.wait()
                    ss[n] = stage_B(n, slot, qslot)
                    if n == 0 and 'S' not in order:
                        do_starts()
                elif ch == 'S':
                    do_starts()
                elif ch == 'W':
                    do_waits()
                elif ch == 'X':
                    stage_X(n, ss.pop(n)); done.add(n)
                elif ch == 'C':
                    gs_ = G0 if first else GS
                    if first and n % gs_ == 0:
                        for cp in kv_copies(i, 'v', n // gs_):
                            cp.wait()
                    if n not in done:
                        stage_X(n, ss.pop(n))
                    if first and n == 0 and i + 1 < NG:
                        x_copy(i + 1).wait()
                    stage_C(n, slot, qslot)
                    if early and n == 0 and i + 1 < NG:
                        xpose_group(i + 1)
                elif ch == 'A':
                    if not last:
                        stage_A(i + 1, 1 - qslot)
                elif ch == 'E':
                    if not first:
                        stage_E(i - 1, 1 - qslot, final=last and NG > 1)
            if 'W' not in order:
                do_waits()

        items = dict(x0=[x_copy(0)], q=w0_copies(wq_hbm, wqbuf, wqsem), o=w0_copies(woT_hbm, wobuf, wosem),
                     **{'k0' + 'abcd'[c_]: kv_copies(0, 'k', c_) for c_ in range(G // G0)}, **{'v0' + 'abcd'[c_]: kv_copies(0, 'v', c_) for c_ in range(G // G0)}, **{'k%d' % t: kv_copies(t, 'k') for t in range(1, PD)}, **{'v%d' % t: kv_copies(t, 'v') for t in range(1, PD)}, w=[cp for n_ in range(NG, WD) for cp in w_copies(n_)],
                     **{'x%d' % g: [x_copy(g)] for g in range(1, NG)})
        parts = [p_.split() for p_ in dorder.split('|')]
        parts += [[]] * (4 - len(parts))
        assert sorted(sum(parts, [])) == sorted(items)
        def issue(k_):
            for nm in parts[k_]:
                for cp in items[nm]:
                    cp.start()
        issue(0)
        wqbuf[:, pl.ds(D, NK * 128 - D), :] = jnp.zeros((HW, NK * 128 - D, Dh), bf16)
        x_copy(0).wait()
        xpose_group(0)
        for cp in w0_copies(wq_hbm, wqbuf, wqsem):
            cp.wait()
        stage_A(0, 0)
        for i_ in range(NS):
            step(i_)
        n1 = N1 if U > 1 else NI - 2
        if 1 + n1 > NS:
            lax.fori_loop(NS, 1 + n1, lambda t, c_: (step(t), c_)[1], 0)
        if U > 1:
            assert (NI - 2 - n1) % U == 0
            for t in range(n1 + 2, n1 + 1 + U):
                for cp in kv_copies(t):
                    cp.wait()
            def body(t, carry):
                i = n1 + 1 + U * t
                for u in range(U - 1):
                    step(i + u, ())
                step(i + U - 1, tuple(range(1, U + 1)))
                return carry
            lax.fori_loop(0, (NI - 2 - n1) // U, body, 0)
        step(NI - 1)
        nwaited = NI - 1 + U
        for t in range(nwaited, NI - 1 + PD):
            for cp in kv_copies(t):
                cp.wait()
        for cp in w_copies(NI - 2 + WD):
            cp.wait()
        stage_E(NI - 1, (NI - 1) % 2, final=True)
        for b in range(B):
            o_copy(b).wait()

    @jax.jit
    def pallas_standalone__gqa_block_cached__near_ridge_kernel(x, k_cache, v_cache, wq, wo):
        xT = x.transpose(0, 2, 1)
        woT = wo.T
        anyspec = pl.BlockSpec(memory_space=pl.ANY)
        outT = pl.pallas_call(
            kernel,
            in_specs=[anyspec] * 5,
            out_specs=anyspec,
            out_shape=jax.ShapeDtypeStruct((B, D, Sq), x.dtype),
            scratch_shapes=[
                pltpu.VMEM((B, D, Sq), bf16),
                pltpu.VMEM((NK, B * Sq, 128), bf16),
                pltpu.VMEM((NBUF, G, Sk, Dh), bf16),
                pltpu.VMEM((NBUF, G, Sk, Dh), bf16),
                pltpu.VMEM((HW, NK * 128, Dh), bf16),
                pltpu.VMEM((HW, D, Dh), bf16),
                pltpu.VMEM((2, G, 2 * Sq, Dh), bf16),
                pltpu.VMEM((2, G, 2 * Sq, Dh), bf16),
                pltpu.VMEM((B, D, Sq), f32),
                pltpu.VMEM((B, D, Sq), bf16),
                pltpu.VMEM((2, Sk // 128, 2 * Sq, 128), bf16),
                pltpu.VMEM((2, KS, 2 * Sq, Dh), f32),
                pltpu.SemaphoreType.DMA((2, G)),
                pltpu.SemaphoreType.DMA((NG,)),
                pltpu.SemaphoreType.DMA((NBUF, G // GS)),
                pltpu.SemaphoreType.DMA((NBUF, G // GS)),
                pltpu.SemaphoreType.DMA((10,)),
                pltpu.SemaphoreType.DMA((10,)),
                pltpu.SemaphoreType.DMA((B,)),
            ],
            compiler_params=pltpu.CompilerParams(vmem_limit_bytes=vmem * 1024 * 1024),
        )(xT, k_cache, v_cache, wq, woT)
        return outT.transpose(0, 2, 1)
    return pallas_standalone__gqa_block_cached__near_ridge_kernel


pallas_standalone__gqa_block_cached__near_ridge_kernel = _build()
```
